```python
import os as _os
_os.environ.setdefault('JAX_PLATFORMS', 'cpu')
import jax
import jax.numpy as jnp

def _softmax(x, axis=-1):
    return jax.nn.softmax(x, axis=axis)

def _gelu(x):
    return jax.nn.gelu(x, approximate=True)

def _silu(x):
    return jax.nn.silu(x)

def _sigmoid(x):
    return jax.nn.sigmoid(x)

def _layernorm(x, axis=-1, eps=1e-05):
    m = jnp.mean(x, axis=axis, keepdims=True)
    v = jnp.var(x, axis=axis, keepdims=True)
    return (x - m) / jnp.sqrt(v + eps)

def _scatter_add(tgt, idx, src, axis=0):
    return tgt.at[idx].add(src)

def _segment_sum(src, seg, n):
    return jax.ops.segment_sum(src, seg, n)

class _Rng:

    def __init__(self, key):
        self._k = key

    def _next(self):
        self._k, sub = jax.random.split(self._k)
        return sub

    def normal(self, shape):
        return jax.random.normal(self._next(), shape, dtype=jnp.bfloat16)

    def randint(self, lo, hi, shape):
        return jax.random.randint(self._next(), shape, lo, hi, dtype=jnp.int32)

    def uniform(self, shape, lo=0.0, hi=1.0):
        return jax.random.uniform(self._next(), shape, jnp.bfloat16, lo, hi)

    def permutation(self, n):
        return jax.random.permutation(self._next(), n)
kernel_name = 'adaLN_cond__sliding_block__dense_activation_silu__prompt'

def setup_inputs():
    _rng = _Rng(jax.random.key(int.from_bytes(__import__("os").urandom(4), "little")))
    _w = lambda a: (lambda t: t.astype(jnp.bfloat16) if jnp.issubdtype(t.dtype, jnp.floating) else t)(jnp.asarray(a))

    def _A_setup():
        B, S, D = (1, 2048, 512)
        return {'x': _w((lambda *s: _rng.normal(s) * 0.05)(B, S, D)), 'wqkv': _w((lambda *s: _rng.normal(s) * 0.05)(D, 3 * D)), 'wo': _w((lambda *s: _rng.normal(s) * 0.05)(D, D))}
    _A_in = _A_setup()

    def _B_setup():
        B, S, D, F = (1, 2048, 512, 1792)
        return {'x': _w((lambda *s: _rng.normal(s) * 0.05)(B, S, D)), 'w1': _w((lambda *s: _rng.normal(s) * 0.8)(D, F) * D ** (-0.5)), 'w2': _w((lambda *s: _rng.normal(s) * 0.8)(F, D) * F ** (-0.5))}
    _B_in = _B_setup()
    return {'A_x': _A_in['x'], 'A_wqkv': _A_in['wqkv'], 'A_wo': _A_in['wo'], 'B_x': _B_in['x'], 'B_w1': _B_in['w1'], 'B_w2': _B_in['w2'], 'c': _w((lambda *s: _rng.normal(s) * 0.05)(1, 512) * 8.0), 'w_mod': _w((lambda *s: _rng.normal(s) * 0.05)(512, 6 * 512) * 512 ** (-0.5) * 8.0)}

def reference(A_x, A_wqkv, A_wo, B_x, B_w1, B_w2, c, w_mod):

    def _A_ref(x, wqkv, wo):
        B, S, D = x.shape
        H = 32
        Dh = D // H
        W = 256
        qkv = (lambda x, *d: x.transpose(*d))((x @ wqkv).reshape(B, S, 3, H, Dh), 2, 0, 3, 1, 4)
        q, k, v = (qkv[0], qkv[1], qkv[2])
        scores = jnp.einsum('bhqd,bhkd->bhqk', q, k) * Dh ** (-0.5)
        idx = jnp.arange(S)
        mask = (idx[:, None] - idx[None, :] >= 0) & (idx[:, None] - idx[None, :] < W)
        scores = jnp.where(mask[None, None], scores, -1000000000.0)
        p = _softmax(scores, axis=-1)
        o = jnp.einsum('bhqk,bhkd->bhqd', p, v)
        return (lambda x, *d: x.transpose(*d))(o, 0, 2, 1, 3).reshape(B, S, D) @ wo

    def _B_ref(x, w1, w2):
        h = jnp.einsum('bsd,df->bsf', x, w1)
        h = _silu(h)
        out = jnp.einsum('bsf,fd->bsd', h, w2)
        return out
    x = A_x
    mod = (_silu(c) @ w_mod).reshape(c.shape[0], 6, 1, -1)
    sa, ca, ga, sb, cb, gb = (mod[:, 0].copy(), mod[:, 1].copy(), mod[:, 2].copy(), mod[:, 3].copy(), mod[:, 4].copy(), mod[:, 5].copy())
    h = _layernorm(x, axis=-1) * (1 + ca) + sa
    x = x + ga * _A_ref(h, A_wqkv, A_wo)
    h = _layernorm(x, axis=-1) * (1 + cb) + sb
    x = x + gb * _B_ref(h, B_w1, B_w2)
    return x
```

```python
import functools
import math
import jax
import jax.numpy as jnp
from jax import lax
import jax.experimental.pallas as pl
import jax.experimental.pallas.tpu as pltpu

S = 2048
D = 512
H = 32
DH = 16
W = 256
F = 1792
EPS = 1e-5
NEG = -1e9
LOG2E = 1.4426950408889634

NT = (((1,), (1,)), ((), ()))
bf16 = jnp.bfloat16
f32 = jnp.float32
u32 = jnp.uint32


def _ln(x):
    m = jnp.mean(x, axis=-1, keepdims=True)
    xc = x - m
    v = jnp.mean(xc * xc, axis=-1, keepdims=True)
    return xc * lax.rsqrt(v + EPS)


def _silu(x):
    t = 0.5 * x
    return t * jnp.tanh(t) + t


def pk(x):
    return pltpu.bitcast(x, u32)


def upk(x):
    return pltpu.bitcast(x, bf16)


def make_kernel(TQ=256, G=2, NSLOT=2, IL=16, FIRST=True):
    QB = 128 // G
    WIN = W + QB
    NB = TQ // 128
    NU = 8 // G
    NL = NU * 128

    def kernel(x_ref, wqkv_ref, wo_ref, w1_ref, w2_ref, c_ref, wmod_ref,
               o_ref, mod_scr, k_scr, vT_scr, qT_scr, oT_scr, s_scr):
        i = pl.program_id(0)

        def body(first):
            if first:
                c = c_ref[...].astype(f32)
                sc = c * jax.nn.sigmoid(c)
                sc8 = jnp.broadcast_to(sc, (8, D)).astype(bf16)
                mod_scr[...] = jnp.dot(sc8, wmod_ref[...], preferred_element_type=f32)
                k_scr[0:W // 2, :] = jnp.zeros((W // 2, D), u32)
                vT_scr[0:2] = jnp.zeros((2, D // 2, 128), u32)

            sa = mod_scr[0:1, 0 * D:1 * D]
            ca = mod_scr[0:1, 1 * D:2 * D]
            ga = mod_scr[0:1, 2 * D:3 * D]
            sb = mod_scr[0:1, 3 * D:4 * D]
            cb = mod_scr[0:1, 4 * D:5 * D]
            gb = mod_scr[0:1, 5 * D:6 * D]

            x = x_ref[...].astype(f32)
            h = (_ln(x) * (1.0 + ca) + sa).astype(bf16)

            r0h = 0 if first else pl.multiple_of(i * (TQ // 2), TQ // 2)
            ib = 0 if first else i * NB
            qkv = jnp.dot(h, wqkv_ref[...], preferred_element_type=f32)
            k_scr[pl.ds(W // 2 + r0h, TQ // 2), :] = pk(qkv[:, D:2 * D].astype(bf16))
            qT = (qkv[:, 0:D] * (DH ** -0.5 * LOG2E)).T
            if G == 1:
                qT_scr[0] = pk(qT.astype(bf16))
            else:
                lane = lax.broadcasted_iota(jnp.int32, (16, 128), 1)
                lo = lane < 64
                for b in range(NB):
                    for hh in range(H):
                        t = qT[hh * 16:(hh + 1) * 16, b * 128:(b + 1) * 128].astype(bf16)
                        t = pk(t)
                        lo8 = lo[0:8]
                        z = jnp.zeros_like(t)
                        if hh % 2 == 1:
                            t = pltpu.roll(t, 64, 1)
                            qa = jnp.where(lo8, z, t); qb = jnp.where(lo8, t, z)
                        else:
                            qa = jnp.where(lo8, t, z); qb = jnp.where(lo8, z, t)
                        qT_scr[0, hh * 8:(hh + 1) * 8, b * 128:(b + 1) * 128] = qa
                        qT_scr[1, hh * 8:(hh + 1) * 8, b * 128:(b + 1) * 128] = qb
            vT = pk(qkv[:, 2 * D:3 * D].T.astype(bf16))
            for b in range(NB):
                vT_scr[ib + 2 + b] = vT[:, b * 128:(b + 1) * 128]

            row = lax.broadcasted_iota(jnp.int32, (QB, 128), 0)
            col = lax.broadcasted_iota(jnp.int32, (QB, 128), 1)
            tri = row <= (col % QB)

            gus = [(b, a, g) for b in range(NB) for g in range(4) for a in range(G)]

            def nskip(n):
                b, a, g = gus[n]
                if not first:
                    return 0
                q0 = b * 128 + a * QB
                return max(0, W - q0)

            def stage_a(n):
                b, a, g = gus[n]
                sk = nskip(n)
                q0h = r0h + (b * 128 + a * QB) // 2
                kw = upk(k_scr[pl.ds(q0h + sk // 2, (WIN - sk) // 2), g * 128:(g + 1) * 128])
                if IL and sk == 0:
                    parts = []
                    for c0 in range(0, QB, IL):
                        parts.append(kw[c0:c0 + IL]); parts.append(kw[W + c0:W + c0 + IL])
                    parts.append(kw[QB:W])
                    kw = jnp.concatenate(parts, axis=0)
                cols = []
                for u in range(NU):
                    r_lo = u * G * 8
                    qh = qT_scr[a, g * 64 + r_lo:g * 64 + r_lo + G * 8, b * 128:(b + 1) * 128]
                    parts = []
                    if r_lo > 0:
                        parts.append(jnp.zeros((r_lo, 128), u32))
                    parts.append(qh)
                    if r_lo + G * 8 < 64:
                        parts.append(jnp.zeros((64 - r_lo - G * 8, 128), u32))
                    cols.append(jnp.concatenate(parts, axis=0))
                wq = upk(jnp.concatenate(cols, axis=1))
                s = jnp.dot(kw, wq, preferred_element_type=f32)
                ms = []
                for u in range(NU):
                    su = s[:, u * 128:(u + 1) * 128]
                    if sk == 0:
                        if IL:
                            frst = jnp.concatenate([su[2 * c0:2 * c0 + IL] for c0 in range(0, QB, IL)], axis=0)
                            last = jnp.concatenate([su[2 * c0 + IL:2 * c0 + 2 * IL] for c0 in range(0, QB, IL)], axis=0)
                            mid = su[2 * QB:]
                        else:
                            frst = su[0:QB]; mid = su[QB:W]; last = su[W:WIN]
                        merged = jnp.where(tri, last, frst)
                        sm = jnp.concatenate([merged, mid], axis=0)
                    else:
                        nr = WIN - sk
                        last = jnp.where(tri, su[nr - QB:nr], NEG)
                        sm = jnp.concatenate([last, su[0:nr - QB]], axis=0) if nr > QB else last
                    ms.append(jnp.max(sm, axis=0, keepdims=True))
                    s_scr[n % NSLOT, 0:sm.shape[0], u * 128:(u + 1) * 128] = sm
                return ms

            def stage_b(n, ms, prev):
                b, a, g = gus[n]
                sk = nskip(n)
                nr = W if sk == 0 else WIN - sk
                outs = []
                for u in range(NU):
                    sm = s_scr[n % NSLOT, 0:nr, u * 128:(u + 1) * 128]
                    p = jnp.exp2(sm - ms[u])
                    l = jnp.sum(p, axis=0, keepdims=True)
                    pm = p[0:QB]
                    if sk == 0:
                        pp = [jnp.where(tri, 0.0, pm), p[QB:W], jnp.where(tri, pm, 0.0)]
                    else:
                        pp = ([p[QB:nr]] if nr > QB else []) + [pm]
                    tail = 128 - QB - a * QB
                    tot = sum(t.shape[0] for t in pp) + tail
                    nt = -(-tot // 128)
                    head = nt * 128 - tot
                    if head: pp = [jnp.zeros((head, 128), f32)] + pp
                    if tail: pp = pp + [jnp.zeros((tail, 128), f32)]
                    pfull = jnp.concatenate(pp, axis=0).astype(bf16)
                    r_lo = g * 64 + u * G * 8
                    vw = upk(jnp.concatenate(
                        [vT_scr[ib + b + t, r_lo:r_lo + G * 8, :] for t in range(3 - nt, 3)], axis=1))
                    oT = jnp.dot(vw, pfull, preferred_element_type=f32) * (1.0 / l)
                    ro = 2 * r_lo
                    if G == 1:
                        oT_scr[ro:ro + 16, b * 128:(b + 1) * 128] = oT
                    else:
                        if a == 0:
                            outs.append(oT)
                        else:
                            lane = lax.broadcasted_iota(jnp.int32, (16, 128), 1)
                            lo = lane < 64
                            o0 = prev[u]
                            e = jnp.where(lo, o0[0:16], oT[0:16])
                            od = jnp.where(lo, oT[16:32], o0[16:32])
                            od = pltpu.roll(od, 64, 1)
                            oT_scr[ro:ro + 16, b * 128:(b + 1) * 128] = e
                            oT_scr[ro + 16:ro + 32, b * 128:(b + 1) * 128] = od
                return outs

            ms_next = stage_a(0)
            prev = None
            for n in range(len(gus)):
                ms = ms_next
                if n + 1 < len(gus):
                    ms_next = stage_a(n + 1)
                prev = stage_b(n, ms, prev)

            o = oT_scr[...].T.astype(bf16)
            attn = jnp.dot(o, wo_ref[...], preferred_element_type=f32)
            x1 = x + ga * attn
            h2 = (_ln(x1) * (1.0 + cb) + sb).astype(bf16)
            a = jnp.dot(h2, w1_ref[...], preferred_element_type=f32)
            a = _silu(a).astype(bf16)
            y = jnp.dot(a, w2_ref[...], preferred_element_type=f32)
            o_ref[...] = (x1 + gb * y).astype(o_ref.dtype)

        if FIRST:
            pl.when(i == 0)(lambda: body(True))
            pl.when(i > 0)(lambda: body(False))
        else:
            body(False)

    def fn(A_x, A_wqkv, A_wo, B_x, B_w1, B_w2, c, w_mod):
        x = A_x.reshape(S, D)
        const = lambda i: (0, 0)
        out = pl.pallas_call(
            kernel,
            grid=(S // TQ,),
            in_specs=[
                pl.BlockSpec((TQ, D), lambda i: (i, 0)),
                pl.BlockSpec((D, 3 * D), const),
                pl.BlockSpec((D, D), const),
                pl.BlockSpec((D, F), const),
                pl.BlockSpec((F, D), const),
                pl.BlockSpec((1, D), const),
                pl.BlockSpec((D, 6 * D), const),
            ],
            out_specs=pl.BlockSpec((TQ, D), lambda i: (i, 0)),
            out_shape=jax.ShapeDtypeStruct((S, D), bf16),
            scratch_shapes=[
                pltpu.VMEM((8, 6 * D), f32),
                pltpu.VMEM(((S + W) // 2, D), u32),
                pltpu.VMEM((S // 128 + 2, D // 2, 128), u32),
                pltpu.VMEM((G, D // 2, TQ), u32),
                pltpu.VMEM((D, TQ), f32),
                pltpu.VMEM((NSLOT, W, NL), f32),
            ],
            compiler_params=pltpu.CompilerParams(
                dimension_semantics=("arbitrary",),
                vmem_limit_bytes=100 * 2**20),
            name="fused",
        )(x, A_wqkv, A_wo, B_w1, B_w2, c, w_mod)
        return out.reshape(1, S, D)
    return fn


_impl = make_kernel(G=2)


@jax.jit
def pallas_adaLN_cond__sliding_block__dense_activation_silu__prompt_kernel(
    A_x: jax.Array,
    A_wqkv: jax.Array,
    A_wo: jax.Array,
    B_x: jax.Array,
    B_w1: jax.Array,
    B_w2: jax.Array,
    c: jax.Array,
    w_mod: jax.Array,
):
    return _impl(A_x, A_wqkv, A_wo, B_x, B_w1, B_w2, c, w_mod)
```

```python
import functools
import jax
import jax.numpy as jnp
from jax import lax
import jax.experimental.pallas as pl
import jax.experimental.pallas.tpu as pltpu

S = 2048
D = 512
DH = 16
W = 256
F = 1792
EPS = 1e-5
NEG = -1e9
LOG2E = 1.4426950408889634

bf16 = jnp.bfloat16
f32 = jnp.float32
u32 = jnp.uint32

TQ = 256
NS = S // TQ
NB = TQ // 128
HQ = TQ // 2
SL = 8
QS = 128 // SL
WIN = W + QS
HS = QS // 2
NH = (SL - 1) * HS
BITS = (4, 2, 1)
KOFF = 64
NSLOT = 6
NW1A = 7

ORDER_FIRST = (
    "aaaQwaa..Q.a.Q..Q..QQwa..a..Q..a..a..Q..a..a..Q..b..0b..b..Q..b..Q..1b..b..Q.Q.Q..Q..Q..Qw"
    "b..............mQ..mf..mf.3mf.mQ.mf.2mb.mbmQ..mb.mb.mb.Q.f.f.f.Q.f.F.F.Q.f.Q..fwf..mf..mQ.m"
    "fmF..F.Q.fF..F.Q.f.F.F.Q.f.F.F.Q.f.F.F.Q.f.F.F.Q.f.F.F.Q.f.f..f.f.f")
ORDER_STEADY = (
    "ffffaaaaQaa.a.Q.f.A.A.Q.f.F.F.Q.a.F.F.Q.f.f.a.Q.f.f.a.Q.f.F.F.Q.f.A.A.Q.f.f.f.Q.f.F.F.Q.f.F.F.Q."
    "b.F.F.Q.f.b.f.Q.b.f.f.Q.b.B.B.Q.f.F.F.Q.f.f.f.Q.g.g..Q.g.g.b.Q.b.B.B.Q.g.b.g.Q.g.g.b.Q.g.G.G.Q."
    "b.G.G.Q.g.B.B.Q.g.g.g.Q.g.G.G.Q.g.G.G.Q.g.G.G.Q.g.G.G.Q.g.G.G.Q.g.g..g.g.ggg")


def _ln(x):
    m = jnp.mean(x, axis=-1, keepdims=True)
    xc = x - m
    v = jnp.mean(xc * xc, axis=-1, keepdims=True)
    return xc * lax.rsqrt(v + EPS)


def _silu(x):
    t = 0.5 * x
    return t * jnp.tanh(t) + t


def pk(x):
    return pltpu.bitcast(x, u32)


def upk(x):
    return pltpu.bitcast(x, bf16)


def dot(a, b):
    return jnp.dot(a, b, preferred_element_type=f32)


def butterfly_meta():
    arrs = [[(p, 0) for p in range(SL)]]
    for d in BITS:
        nxt = []
        for X in arrs:
            Y = [(X[(p - d) % SL][0], X[(p - d) % SL][1] + d) for p in range(SL)]
            nxt.append([Y[p] if p & d else X[p] for p in range(SL)])
            nxt.append([X[p] if p & d else Y[p] for p in range(SL)])
        arrs = nxt
    meta = []
    for X in arrs:
        assert len({c for c, _ in X}) == 1 and sorted(s for _, s in X) == list(range(SL))
        meta.append((X[0][0], [s for _, s in X]))
    assert sorted(c for c, _ in meta) == list(range(SL))
    return meta


META = butterfly_meta()
SHIFTS = dict(META)
GUS = [(g, b, hf) for g in range(4) for b in range(NB) for hf in range(2)]
NG = len(GUS)


class Blk:
    def __init__(self, off):
        self.off = off


class Lhs:
    def __init__(self, src):
        self.src = src
        self.cache = {}

    def get(self, part):
        if part not in self.cache:
            x = self.src
            if part is not None:
                n = x.shape[0] // 2
                x = x[part * n:(part + 1) * n]
            self.cache[part] = upk(x) if x.dtype == u32 else x.astype(bf16)
        return self.cache[part]


def check_order(order, first, nslot=NSLOT, nw1a=NW1A):
    cnt = dict(a=0, b=0, f=0, g=0)
    half = dict(a=False, b=False, f=False, g=False)
    nq = npv = nm = 0
    nw = 3 if first else 99
    skew = set() if first else {0, 1, 2, 3}
    for ch in order:
        lo = ch.lower()
        if lo in cnt and ch != 'Q':
            j = cnt[lo]
            assert ch != lo or not half[lo]
            if lo in 'ab':
                assert j < 12 and nw > (2, 3, 4, 4)[j // 3] and (lo == 'a' or nw > 4)
                assert lo == 'a' or j % 3 != 1 or (j // 3 in skew and cnt['a'] > j)
            else:
                assert j < 32 and nw > (5 if j < 4 + nw1a else 6)
                if first or lo == 'g':
                    assert npv >= 4 * NG
                if first:
                    assert nm > (j if j < 4 else 11 if j < 18 else 12 + 2 * ((j - 18) // 7) + ((j - 18) % 7) // 4)
                elif lo == 'f' and j == 0:
                    assert npv < 4 * NG + 15
            if ch == lo or half[lo]:
                cnt[lo] += 1
                half[lo] = False
            else:
                half[lo] = True
        elif ch == 'Q':
            assert nq < 2 * NG and cnt['ab'[nq // NG]] > 3 * GUS[nq % NG][0] + 1
            assert npv >= 4 * (nq - nslot + 1)
            nq += 1
        elif ch == '.':
            assert npv < 4 * nq and cnt['ab'[npv // (4 * NG)]] > 3 * GUS[(npv // 4) % NG][0] + 2
            npv += 1
        elif ch == 'w':
            nw += 1
        elif ch == 'm':
            assert nw > (5 if nm < 12 else 6)
            nm += 1
        else:
            assert int(ch) not in skew and cnt['a'] > 3 * int(ch) + 1
            skew.add(int(ch))
    assert cnt == dict(a=12, b=12, f=32, g=0 if first else 32) and nq == 2 * NG and npv == 8 * NG
    assert not first or (nw == 7 and nm == 16 and len(skew) == 4)


def make_kernel(order_first=ORDER_FIRST, order_steady=ORDER_STEADY, interpret=False):
    check_order(order_first, True)
    check_order(order_steady, False)

    def kernel(x_hbm, wqkv_hbm, wo_hbm, w1_hbm, w2_hbm, c_hbm, wmod_hbm, out_hbm,
               mod_scr, k_scr, kh_scr, kn_scr, vT_scr, qT_scr, oT_scr, s_scr, o_scr,
               x_v, out_v, wqkv_ref, wo_ref, w1_ref, w2_ref, c_ref, wmod_ref, fence, sem, sem_o):
        P = functools.partial
        step = pl.program_id(0)
        cp = pltpu.make_async_copy

        def dma_groups():
            def cols(src, dst, c0, c1, s):
                return cp(src.at[:, c0:c1], dst.at[:, c0:c1], sem.at[s])

            def qkv(c0, c1, s):
                return [cols(wqkv_hbm, wqkv_ref, t * D + c0, t * D + c1, s) for t in range(3)]
            return [
                [cp(x_hbm.at[0], x_v.at[0], sem.at[0])],
                [cp(c_hbm, c_ref, sem.at[1]), cols(wmod_hbm, wmod_ref, 0, 2 * D, 1)],
                qkv(0, 128, 2),
                qkv(128, 256, 3),
                qkv(256, 512, 4) + [cp(x_hbm.at[1], x_v.at[1], sem.at[4])],
                [cp(wo_hbm, wo_ref, sem.at[5]), cols(wmod_hbm, wmod_ref, 2 * D, 5 * D, 5),
                 cols(w1_hbm, w1_ref, 0, NW1A * 128, 5)],
                [cols(w1_hbm, w1_ref, NW1A * 128, F, 6), cp(w2_hbm, w2_ref, sem.at[6]),
                 cols(wmod_hbm, wmod_ref, 5 * D, 6 * D, 6)],
                [cp(x_hbm.at[2:NS], x_v.at[2:NS], sem.at[7])],
            ]

        def cp_out(i, c0=0, nc=D):
            return cp(out_v.at[i, :, c0:c0 + nc], out_hbm.at[i, :, c0:c0 + nc], sem_o)

        def region(kind):
            V = {}

            def silu_c():
                if 'sc' not in V:
                    c = c_ref[...].astype(f32)
                    V['sc'] = jnp.broadcast_to(c * jax.nn.sigmoid(c), (8, D)).astype(bf16)
                return V['sc']

            def mod(j, lo=0, hi=D):
                return mod_scr[0:1, j * D + lo:j * D + hi]

            def mod_chunk(j):
                mod_scr[:, j * 128:(j + 1) * 128] = dot(silu_c(), wmod_ref[:, j * 128:(j + 1) * 128])

            def lane_slot(nr):
                return lax.broadcasted_iota(jnp.int32, (nr, 128), 1) // QS

            tri = (lax.broadcasted_iota(jnp.int32, (QS, 128), 0)
                   <= lax.broadcasted_iota(jnp.int32, (QS, 128), 1) % QS)
            bitw = {d: (lane_slot(W) & d) != 0 for d in BITS}
            tri128 = (lax.broadcasted_iota(jnp.int32, (128, 128), 0)
                      <= lax.broadcasted_iota(jnp.int32, (128, 128), 1))

            def lin(i, mult, const):
                if isinstance(i, int):
                    return mult * i + const
                if ('base', mult) not in V:
                    V[('base', mult)] = pl.multiple_of((step - 1) * (2 * mult), mult)
                assert (2 + i.off) * mult + const >= 0
                return V[('base', mult)] + ((2 + i.off) * mult + const)

            def par(i):
                return i % 2 if isinstance(i, int) else i.off % 2

            def is0(i):
                return isinstance(i, int) and i == 0

            def p_ln(i, mid=None):
                xn = _ln(x_v[lin(i, 1, 0)].astype(f32))
                if mid is not None:
                    mid()
                V[('h', par(i))] = Lhs(xn * (1.0 + mod(1)) + mod(0))

            def get_h(i):
                if ('h', par(i)) not in V:
                    p_ln(i)
                return V[('h', par(i))]

            def fin_q(i, g, q):
                qT = (q * (DH ** -0.5 * LOG2E)).T
                qT_scr[par(i), g * 64:(g + 1) * 64, :] = pk(qT.astype(bf16))

            def fin_k(i, g, k):
                kp = pk(k.astype(bf16))
                if is0(i):
                    kn_scr[g] = kp
                else:
                    p_skew(i, g, kp)

            def p_skew(i, g, kp=None):
                if kp is None:
                    kp = kn_scr[g]
                hist = jnp.zeros((NH, 128), u32) if is0(i) else kh_scr[g]
                kh_scr[g] = kp[HQ - NH:HQ]
                arrs = [jnp.concatenate([hist, kp], axis=0)]
                for d in BITS:
                    n = arrs[0].shape[0] - d * HS
                    msk = (lane_slot(n) & d) != 0
                    nxt = []
                    for X in arrs:
                        Y = pltpu.roll(X[d * HS:], d * QS, 1)
                        nxt += [jnp.where(msk, Y, X[0:n]), jnp.where(msk, X[0:n], Y)]
                    arrs = nxt
                for X, (c, _) in zip(arrs, META):
                    k_scr[g * SL + c, pl.ds(lin(i, HQ, KOFF - NH), HQ), :] = X

            def fin_v(i, g, v):
                vT = pk(v.T.astype(bf16))
                for b in range(NB):
                    vT_scr[lin(i, NB, b), g * 64:(g + 1) * 64, :] = vT[:, b * 128:(b + 1) * 128]

            def slab(ref, r0, r1, c0, c1):
                return ref[r0:r1, c0:c1]

            def proj(i):
                return [(P(get_h, i), P(slab, wqkv_ref, 0, D, t * D + g * 128, t * D + (g + 1) * 128), P(fin, i, g))
                        for g in range(4) for t, fin in enumerate((fin_q, fin_k, fin_v))]

            def a_qk0(n, sl_):
                g, b, hf = GUS[n]
                nr = (b + 1) * 128
                kw = upk(kn_scr[g, 0:nr // 2, :])
                z = jnp.zeros((8, 128), u32)
                cols = []
                for u in range(4):
                    hl = hf * 4 + u
                    qh = qT_scr[0, (g * 8 + hl) * 8:(g * 8 + hl + 1) * 8, b * 128:(b + 1) * 128]
                    cols.append(jnp.concatenate([qh if p == hl else z for p in range(8)], axis=0))
                s_ = dot(kw, upk(jnp.concatenate(cols, axis=1)))
                ms = []
                for u in range(4):
                    su = s_[:, u * 128:(u + 1) * 128]
                    diag = jnp.where(tri128, su[nr - 128:nr], NEG)
                    sm = diag if b == 0 else jnp.concatenate([su[0:nr - 128], diag], axis=0)
                    ms.append(jnp.max(sm, axis=0, keepdims=True))
                    s_scr[sl_, 0:nr, u * 128:(u + 1) * 128] = sm
                V[('m', sl_)] = ms

            def a_qk(i, n, sl_):
                if is0(i):
                    return a_qk0(n, sl_)
                g, b, hf = GUS[n]
                ms = []
                for u in range(4):
                    c = hf * 4 + u
                    hh = g * 8 + c
                    kw = k_scr[hh, pl.ds(lin(i, HQ, KOFF - W // 2 + b * 64), WIN // 2), :]
                    kw = upk(jnp.concatenate([kw[0:HS], kw[W // 2:W // 2 + HS], kw[HS:W // 2]], axis=0))
                    qh = qT_scr[par(i), hh * 8:(hh + 1) * 8, b * 128:(b + 1) * 128]
                    if ('qmask', c) not in V:
                        V[('qmask', c)] = lane_slot(64) == jnp.concatenate(
                            [jnp.full((8, 128), sh, jnp.int32) for sh in SHIFTS[c]], axis=0)
                    wq = jnp.where(V[('qmask', c)], jnp.concatenate([qh] * SL, axis=0), jnp.zeros((64, 128), u32))
                    su = dot(kw, upk(wq))
                    sm = jnp.concatenate([jnp.where(tri, su[QS:2 * QS], su[0:QS]), su[2 * QS:]], axis=0)
                    ms.append(jnp.max(sm, axis=0, keepdims=True))
                    s_scr[sl_, :, u * 128:(u + 1) * 128] = sm
                V[('m', sl_)] = ms

            def a_pv(i, n, sl_, u):
                g, b, hf = GUS[n]
                m = V[('m', sl_)][u]
                hh = g * 8 + hf * 4 + u
                if is0(i):
                    sx = s_scr[sl_, 0:(b + 1) * 128, u * 128:(u + 1) * 128]
                    tiles = range(b + 1)
                else:
                    sx = s_scr[sl_, :, u * 128:(u + 1) * 128]
                    for d in BITS:
                        sx = jnp.where(bitw[d], jnp.concatenate([sx[W - d * QS:], sx[:W - d * QS]], axis=0), sx)
                    tiles = [lin(i, NB, b - 2 + t) for t in range(3)]
                p = jnp.exp2(sx - m)
                lsum = None
                for c0 in range(0, p.shape[0], 128):
                    part = None
                    for j in range(c0 + 112, c0 - 1, -16):
                        part = p[j:j + 16] if part is None else part + p[j:j + 16]
                    lsum = part if lsum is None else lsum + part
                rl = pl.reciprocal(jnp.sum(lsum, axis=0, keepdims=True), approx=True)
                if not is0(i):
                    pm = p[0:128]
                    p = jnp.concatenate([jnp.where(tri128, 0.0, pm), p[128:256], jnp.where(tri128, pm, 0.0)], axis=0)
                vw = upk(jnp.concatenate([vT_scr[t, hh * 8:(hh + 1) * 8, :] for t in tiles], axis=1))
                oT_scr[hh * 16:(hh + 1) * 16, b * 128:(b + 1) * 128] = dot(vw, p.astype(bf16)) * rl
                if u == 3 and n % 4 == 3:
                    o_scr[par(i), :, g * 128:(g + 1) * 128] = pk(oT_scr[g * 128:(g + 1) * 128, :].T.astype(bf16))

            def ffn(i, r0=0, nr=TQ, T=None):
                T = {} if T is None else T

                def get_o():
                    if 'o' not in T:
                        T['o'] = Lhs(o_scr[par(i), r0 // 2:(r0 + nr) // 2, :])
                        T['x1'] = []
                    return T['o']

                def fin_wo(j, attn):
                    xp = x_v[lin(i, 1, 0), r0:r0 + nr, j * 128:(j + 1) * 128].astype(f32)
                    T['x1'].append(xp + mod(2, j * 128, (j + 1) * 128) * attn)
                    if j == 3 and kind != 'first':
                        get_h2()

                def get_h2():
                    if 'h2' not in T:
                        T['h2'] = Lhs(_ln(jnp.concatenate(T['x1'], axis=1)) * (1.0 + mod(4)) + mod(3))
                        T['a'] = []
                    return T['h2']

                def fin_w1(j, a):
                    T['a'].append(_silu(a))
                    if j % 4 == 3 or j == 13:
                        T[('ac', j // 4)] = Lhs(jnp.concatenate(T['a'][4 * (j // 4):j + 1], axis=1))

                def fin_w2r(pr, y):
                    T[('y', 2 * pr)] = y[:, 0:128]
                    T[('y', 2 * pr + 1)] = y[:, 128:256]

                def fin_w2(n, c, y):
                    T[('y', n)] = T[('y', n)] + y
                    if c == 2:
                        out_v[lin(i, 1, 0), r0:r0 + nr, n * 128:(n + 1) * 128] = (
                            T['x1'][n] + mod(5, n * 128, (n + 1) * 128) * T[('y', n)]).astype(bf16)
                        if kind == 'last' and n >= 2:
                            cp_out(i, *((0, 384), (384, 128))[n - 2]).start()
                        elif kind != 'last' and n == 3:
                            cp_out(lin(i, 1, 0)).start()

                items = [(get_o, P(slab, wo_ref, 0, D, j * 128, (j + 1) * 128), P(fin_wo, j)) for j in range(4)]
                items += [(get_h2, P(slab, w1_ref, 0, D, j * 128, (j + 1) * 128), P(fin_w1, j)) for j in range(14)]
                for pr in range(2):
                    items.append((P(T.get, ('ac', 3)), P(slab, w2_ref, 1536, F, pr * 256, (pr + 1) * 256),
                                  P(fin_w2r, pr)))
                    items += [(P(T.get, ('ac', c)), P(slab, w2_ref, c * 512, (c + 1) * 512, n * 128, (n + 1) * 128),
                               P(fin_w2, n, c)) for n in (2 * pr, 2 * pr + 1) for c in range(3)]
                return items

            def run(item):
                lhs, w, fin = item
                fin(dot(lhs().get(None), w()))

            def emit(order, blocks, streams, extra):
                stash = {}
                nq = npv = 0
                for ch in order:
                    if ch == 'Q':
                        a_qk(blocks[nq // NG], nq % NG, nq % NSLOT)
                        nq += 1
                    elif ch == '.':
                        q, u = divmod(npv, 4)
                        a_pv(blocks[q // NG], q % NG, q % NSLOT, u)
                        npv += 1
                    elif ch in streams:
                        run(streams[ch].pop(0))
                    elif ch.lower() in streams:
                        lhs, w, fin = streams[ch.lower()][0]
                        if ch not in stash:
                            stash[ch] = dot(lhs().get(0), w())
                        else:
                            streams[ch.lower()].pop(0)
                            fin(jnp.concatenate([stash.pop(ch), dot(lhs().get(1), w())], axis=0))
                    else:
                        extra[ch].pop(0)()

            if kind == 'first':
                groups = dma_groups()
                for grp in groups:
                    for c_ in grp:
                        c_.start()
                        pl.semaphore_signal(fence, 1)
                        pl.semaphore_wait(fence, 1)

                def wait(k):
                    for c_ in groups[k]:
                        c_.wait()

                def mod_a():
                    wait(1)
                    for j in range(8):
                        mod_chunk(j)

                wait(0)
                p_ln(0, mod_a)
                V[('h', 0)].get(None)
                wait(2)
                extra = {str(g): [P(p_skew, 0, g)] for g in range(4)}
                extra['w'] = [P(wait, k) for k in range(3, 7)]
                extra['m'] = [P(mod_chunk, j) for j in range(8, 24)]
                emit(order_first, (0, 1), dict(a=proj(0), b=proj(1), f=ffn(0)), extra)
                wait(7)
            elif kind == 'steady':
                bm1, b0, b1 = Blk(-1), Blk(0), Blk(1)
                p_ln(b0)
                emit(order_steady, (b0, b1), dict(a=proj(b0), b=proj(b1), f=ffn(bm1), g=ffn(b0)), {})
            else:
                Ta, Tb, T = {}, {}, {}
                a, b = ffn(NS - 1, 0, 128, Ta), ffn(NS - 1, 128, 128, Tb)
                for item in a[:4] + b[:4] + a[4:7] + b[4:7]:
                    run(item)
                T['h2'] = Lhs(jnp.concatenate([Ta['h2'].src, Tb['h2'].src], axis=0))
                for k in ('x1', 'a'):
                    T[k] = [jnp.concatenate(p, axis=0) for p in zip(Ta[k], Tb[k])]
                for item in ffn(NS - 1, T=T)[7:]:
                    run(item)
                cp(out_v, out_hbm, sem_o).wait()

        pl.when(step == 0)(lambda: region('first'))
        pl.when(jnp.logical_and(step > 0, step < 4))(lambda: region('steady'))
        pl.when(step == 4)(lambda: region('last'))

    def fn(A_x, A_wqkv, A_wo, B_x, B_w1, B_w2, c, w_mod):
        out = pl.pallas_call(
            kernel,
            grid=(5,),
            in_specs=[pl.BlockSpec(memory_space=pl.ANY)] * 7,
            out_specs=pl.BlockSpec(memory_space=pl.ANY),
            out_shape=jax.ShapeDtypeStruct((NS, TQ, D), bf16),
            scratch_shapes=[
                pltpu.VMEM((8, 6 * D), f32),
                pltpu.VMEM((4 * SL, S // 2 + KOFF, 128), u32),
                pltpu.VMEM((4, NH, 128), u32),
                pltpu.VMEM((4, HQ, 128), u32),
                pltpu.VMEM((S // 128, D // 2, 128), u32),
                pltpu.VMEM((2, D // 2, TQ), u32),
                pltpu.VMEM((D, TQ), f32),
                pltpu.VMEM((NSLOT, W, 512), f32),
                pltpu.VMEM((2, HQ, D), u32),
                pltpu.VMEM((NS, TQ, D), bf16),
                pltpu.VMEM((NS, TQ, D), bf16),
                pltpu.VMEM((D, 3 * D), bf16),
                pltpu.VMEM((D, D), bf16),
                pltpu.VMEM((D, F), bf16),
                pltpu.VMEM((F, D), bf16),
                pltpu.VMEM((1, D), bf16),
                pltpu.VMEM((D, 6 * D), bf16),
                pltpu.SemaphoreType.REGULAR,
                pltpu.SemaphoreType.DMA((8,)),
                pltpu.SemaphoreType.DMA,
            ],
            compiler_params=pltpu.CompilerParams(
                dimension_semantics=("arbitrary",),
                vmem_limit_bytes=100 * 2**20),
            name="fused",
            interpret=interpret,
        )(A_x.reshape(NS, TQ, D), A_wqkv, A_wo, B_w1, B_w2, c, w_mod)
        return out.reshape(1, S, D)
    return fn


_impl = make_kernel()


@jax.jit
def pallas_adaLN_cond__sliding_block__dense_activation_silu__prompt_kernel(
    A_x: jax.Array,
    A_wqkv: jax.Array,
    A_wo: jax.Array,
    B_x: jax.Array,
    B_w1: jax.Array,
    B_w2: jax.Array,
    c: jax.Array,
    w_mod: jax.Array,
):
    return _impl(A_x, A_wqkv, A_wo, B_x, B_w1, B_w2, c, w_mod)
```

```python
import functools
import jax
import jax.numpy as jnp
from jax import lax
import jax.experimental.pallas as pl
import jax.experimental.pallas.tpu as pltpu

S = 2048
D = 512
DH = 16
W = 256
F = 1792
EPS = 1e-5
NEG = -1e9
LOG2E = 1.4426950408889634

bf16 = jnp.bfloat16
f32 = jnp.float32
u32 = jnp.uint32

TQ = 256
NS = S // TQ
NB = TQ // 128
HQ = TQ // 2
SL = 8
QS = 128 // SL
WIN = W + QS
HS = QS // 2
NH = (SL - 1) * HS
BITS = (4, 2, 1)
NSLOT = 6
NW1A = 7

ORDER_FIRST = (
    "aaaQQwQ.a.A.A...Q.aQQ.....wQa..a..a...a....Q...a...Q..Qb...0aQ...b.Q.....Q.BB...Q...Q.Q..2.B...B"
    "..1b...b.b.Qwb.mmQm.bm.Fm.Fm.Q.3fm.Fmm.Fm.Q.mmf.b..Q.b.b.F.FQ.f.F.F.Q.f.F.F.Q.FFFF...Q.wfm.fm.Q."
    "m.fm.F..F.f.QF.F.Q.f.FF..Q.F.FF.F.Q.f.F.F.Q.f.F.F.Q.f.F..FfF.Ff.f.f")
ORDER_STEADY = (
    "ffffaaaaQaa.a.Q.f.A.A.Q.f.F.F.Q.a.F.F.Q.f.f.a.Q.f.f.a.Q.f.F.F.Q.f.A.A.Q.f.f.f.Q.f.F.F.Q.f.F.F.Q."
    "b.F.F.Q.f.b.f.Q.b.f.f.Q.b.B.B.Q.f.F.F.Q.f.f.f.Q.g.g..Q.g.g.b.Q.b.B.B.Q.g.b.g.Q.g.g.b.Q.g.G.G.Q.b"
    ".G.G.Q.g.B.B.Q.g.g.g.Q.g.G.G.Q.g.G.G.Q.g.G.G.Q.g.G.G.Q.g.G.G.Q.g.g.g.g.g.gg")


def _ln(x):
    m = jnp.mean(x, axis=-1, keepdims=True)
    xc = x - m
    v = jnp.mean(xc * xc, axis=-1, keepdims=True)
    return xc * lax.rsqrt(v + EPS)


def _silu(x):
    t = 0.5 * x
    return t * jnp.tanh(t) + t


def pk(x):
    return pltpu.bitcast(x, u32)


def upk(x):
    return pltpu.bitcast(x, bf16)


def dot(a, b):
    return jnp.dot(a, b, preferred_element_type=f32)


def butterfly_meta():
    arrs = [[(p, 0) for p in range(SL)]]
    for d in BITS:
        nxt = []
        for X in arrs:
            Y = [(X[(p - d) % SL][0], X[(p - d) % SL][1] + d) for p in range(SL)]
            nxt.append([Y[p] if p & d else X[p] for p in range(SL)])
            nxt.append([X[p] if p & d else Y[p] for p in range(SL)])
        arrs = nxt
    meta = []
    for X in arrs:
        assert len({c for c, _ in X}) == 1 and sorted(s for _, s in X) == list(range(SL))
        meta.append((X[0][0], [s for _, s in X]))
    assert sorted(c for c, _ in meta) == list(range(SL))
    return meta


META = butterfly_meta()
SHIFTS = dict(META)
GUS = [(g, b, hf) for g in range(4) for b in range(NB) for hf in range(2)]
NG = len(GUS)


class Blk:
    def __init__(self, off):
        self.off = off


class Lhs:
    def __init__(self, src):
        self.src = src
        self.cache = {}

    def get(self, part):
        if part not in self.cache:
            x = self.src
            if part is not None:
                n = x.shape[0] // 2
                x = x[part * n:(part + 1) * n]
            self.cache[part] = upk(x) if x.dtype == u32 else x.astype(bf16)
        return self.cache[part]


def check_order(order, first, nslot=NSLOT, nw1a=NW1A):
    cnt = dict(a=0, b=0, f=0, g=0)
    half = dict(a=False, b=False, f=False, g=False)
    nq = npv = nm = 0
    nw = 3 if first else 99
    skew = set() if first else {0, 1, 2, 3}
    for ch in order:
        lo = ch.lower()
        if lo in cnt and ch != 'Q':
            j = cnt[lo]
            assert ch != lo or not half[lo]
            if lo in 'ab':
                assert j < 12 and nw > (2, 3, 4, 4)[j // 3] and (lo == 'a' or nw > 4)
                assert lo == 'a' or j % 3 != 1 or (j // 3 in skew and cnt['a'] > j)
            else:
                assert j < 32 and nw > (5 if j < 4 + nw1a else 6)
                if first or lo == 'g':
                    assert npv >= 4 * NG
                if first:
                    assert nm > (j if j < 4 else 11 if j < 18 else 12 + 2 * ((j - 18) // 7) + ((j - 18) % 7) // 4)
                elif lo == 'f' and j == 0:
                    assert npv < 4 * NG + 15
            if ch == lo or half[lo]:
                cnt[lo] += 1
                half[lo] = False
            else:
                half[lo] = True
        elif ch == 'Q':
            assert nq < 2 * NG and cnt['ab'[nq // NG]] > 3 * GUS[nq % NG][0] + 1
            assert npv >= 4 * (nq - nslot + 1)
            nq += 1
        elif ch == '.':
            assert npv < 4 * nq and cnt['ab'[npv // (4 * NG)]] > 3 * GUS[(npv // 4) % NG][0] + 2
            npv += 1
        elif ch == 'w':
            nw += 1
        elif ch == 'm':
            assert nw > (5 if nm < 12 else 6)
            nm += 1
        else:
            assert int(ch) not in skew and cnt['a'] > 3 * int(ch) + 1
            skew.add(int(ch))
    assert cnt == dict(a=12, b=12, f=32, g=0 if first else 32) and nq == 2 * NG and npv == 8 * NG
    assert not first or (nw == 7 and nm == 16 and len(skew) == 4)


def make_kernel(order_first=ORDER_FIRST, order_steady=ORDER_STEADY, interpret=False):
    check_order(order_first, True)
    check_order(order_steady, False)

    def kernel(x_hbm, wqkv_hbm, wo_hbm, w1_hbm, w2_hbm, c_hbm, wmod_hbm, out_hbm,
               mod_scr, k_scr, kh_scr, kn_scr, vT_scr, qT_scr, oT_scr, s_scr, o_scr,
               x_v, out_v, wqkv_ref, wo_ref, w1_ref, w2_ref, c_ref, wmod_ref, fence, sem, sem_o):
        P = functools.partial
        step = pl.program_id(0)
        cp = pltpu.make_async_copy

        def dma_groups():
            def cols(src, dst, c0, c1, s):
                return cp(src.at[:, c0:c1], dst.at[:, c0:c1], sem.at[s])

            def qkv(c0, c1, s):
                return [cols(wqkv_hbm, wqkv_ref, t * D + c0, t * D + c1, s) for t in range(3)]
            return [
                [cp(x_hbm.at[0], x_v.at[0], sem.at[0])],
                [cp(c_hbm, c_ref, sem.at[1]), cols(wmod_hbm, wmod_ref, 0, 2 * D, 1)],
                qkv(0, 128, 2),
                qkv(128, 256, 3),
                qkv(256, 512, 4) + [cp(x_hbm.at[1], x_v.at[1], sem.at[4])],
                [cp(wo_hbm, wo_ref, sem.at[5]), cols(wmod_hbm, wmod_ref, 2 * D, 5 * D, 5),
                 cols(w1_hbm, w1_ref, 0, NW1A * 128, 5)],
                [cols(w1_hbm, w1_ref, NW1A * 128, F, 6), cp(w2_hbm, w2_ref, sem.at[6]),
                 cols(wmod_hbm, wmod_ref, 5 * D, 6 * D, 6)],
                [cp(x_hbm.at[2:NS], x_v.at[2:NS], sem.at[7])],
            ]

        def cp_out(i, c0=0, nc=D, r0=0, nr=TQ):
            return cp(out_v.at[i, r0:r0 + nr, c0:c0 + nc], out_hbm.at[i, r0:r0 + nr, c0:c0 + nc], sem_o)

        def region(kind):
            V = {}

            def silu_c():
                if 'sc' not in V:
                    c = c_ref[...].astype(f32)
                    V['sc'] = jnp.broadcast_to(c * jax.nn.sigmoid(c), (8, D)).astype(bf16)
                return V['sc']

            def mod(j, lo=0, hi=D):
                return mod_scr[0:1, j * D + lo:j * D + hi]

            def mod_chunk(j):
                mod_scr[:, j * 128:(j + 1) * 128] = dot(silu_c(), wmod_ref[:, j * 128:(j + 1) * 128])

            def lane_slot(nr):
                return lax.broadcasted_iota(jnp.int32, (nr, 128), 1) // QS

            tri = (lax.broadcasted_iota(jnp.int32, (QS, 128), 0)
                   <= lax.broadcasted_iota(jnp.int32, (QS, 128), 1) % QS)
            bitw = {d: (lane_slot(W) & d) != 0 for d in BITS}
            tri128 = (lax.broadcasted_iota(jnp.int32, (128, 128), 0)
                      <= lax.broadcasted_iota(jnp.int32, (128, 128), 1))

            def lin(i, mult, const):
                if isinstance(i, int):
                    return mult * i + const
                if ('base', mult) not in V:
                    V[('base', mult)] = pl.multiple_of((step - 1) * (2 * mult), mult)
                assert (2 + i.off) * mult + const >= 0
                return V[('base', mult)] + ((2 + i.off) * mult + const)

            def par(i):
                return i % 2 if isinstance(i, int) else i.off % 2

            def is0(i):
                return isinstance(i, int) and i == 0

            def p_ln(i, mid=None):
                xn = _ln(x_v[lin(i, 1, 0)].astype(f32))
                if mid is not None:
                    mid()
                V[('h', par(i))] = Lhs(xn * (1.0 + mod(1)) + mod(0))

            def get_h(i):
                if ('h', par(i)) not in V:
                    p_ln(i)
                return V[('h', par(i))]

            def fin_q(i, g, q):
                qT = (q * (DH ** -0.5 * LOG2E)).T
                qT_scr[par(i), g * 64:(g + 1) * 64, :] = pk(qT.astype(bf16))

            def fin_k(i, g, k):
                kp = pk(k.astype(bf16))
                if is0(i):
                    kn_scr[g] = kp
                else:
                    p_skew(i, g, kp)

            def p_skew(i, g, kp=None):
                if kp is None:
                    kp = kn_scr[g]
                arrs = [kp if is0(i) else jnp.concatenate([kh_scr[g], kp], axis=0)]
                kh_scr[g] = kp[HQ - NH:HQ]
                for d in BITS:
                    n = arrs[0].shape[0] - d * HS
                    msk = (lane_slot(n) & d) != 0
                    nxt = []
                    for X in arrs:
                        Y = pltpu.roll(X[d * HS:], d * QS, 1)
                        nxt += [jnp.where(msk, Y, X[0:n]), jnp.where(msk, X[0:n], Y)]
                    arrs = nxt
                for X, (c, _) in zip(arrs, META):
                    k_scr[g * SL + c, pl.ds(0 if is0(i) else lin(i, HQ, -NH), X.shape[0]), :] = X

            def fin_v(i, g, v):
                vT = pk(v.T.astype(bf16))
                for b in range(NB):
                    vT_scr[lin(i, NB, b), g * 64:(g + 1) * 64, :] = vT[:, b * 128:(b + 1) * 128]

            def slab(ref, r0, r1, c0, c1):
                return ref[r0:r1, c0:c1]

            def proj(i):
                return [(P(get_h, i), P(slab, wqkv_ref, 0, D, t * D + g * 128, t * D + (g + 1) * 128), P(fin, i, g))
                        for g in range(4) for t, fin in enumerate((fin_q, fin_k, fin_v))]

            def a_qk0(n, sl_):
                g, b, hf = GUS[n]
                nr = (b + 1) * 128
                kw = upk(kn_scr[g, 0:nr // 2, :])
                z = jnp.zeros((8, 128), u32)
                cols = []
                for u in range(4):
                    hl = hf * 4 + u
                    qh = qT_scr[0, (g * 8 + hl) * 8:(g * 8 + hl + 1) * 8, b * 128:(b + 1) * 128]
                    cols.append(jnp.concatenate([qh if p == hl else z for p in range(8)], axis=0))
                s_ = dot(kw, upk(jnp.concatenate(cols, axis=1)))
                ms = []
                for u in range(4):
                    su = s_[:, u * 128:(u + 1) * 128]
                    diag = jnp.where(tri128, su[nr - 128:nr], NEG)
                    sm = diag if b == 0 else jnp.concatenate([su[0:nr - 128], diag], axis=0)
                    ms.append(jnp.max(sm, axis=0, keepdims=True))
                    s_scr[sl_, 0:nr, u * 128:(u + 1) * 128] = sm
                V[('m', sl_)] = ms

            def a_qk(i, n, sl_):
                if is0(i):
                    return a_qk0(n, sl_)
                g, b, hf = GUS[n]
                ms = []
                for u in range(4):
                    c = hf * 4 + u
                    hh = g * 8 + c
                    kw = k_scr[hh, pl.ds(lin(i, HQ, b * 64 - W // 2), WIN // 2), :]
                    kw = upk(jnp.concatenate([kw[0:HS], kw[W // 2:W // 2 + HS], kw[HS:W // 2]], axis=0))
                    qh = qT_scr[par(i), hh * 8:(hh + 1) * 8, b * 128:(b + 1) * 128]
                    if ('qmask', c) not in V:
                        V[('qmask', c)] = lane_slot(64) == jnp.concatenate(
                            [jnp.full((8, 128), sh, jnp.int32) for sh in SHIFTS[c]], axis=0)
                    wq = jnp.where(V[('qmask', c)], jnp.concatenate([qh] * SL, axis=0), jnp.zeros((64, 128), u32))
                    su = dot(kw, upk(wq))
                    sm = jnp.concatenate([jnp.where(tri, su[QS:2 * QS], su[0:QS]), su[2 * QS:]], axis=0)
                    ms.append(jnp.max(sm, axis=0, keepdims=True))
                    s_scr[sl_, :, u * 128:(u + 1) * 128] = sm
                V[('m', sl_)] = ms

            def a_pv(i, n, sl_, u):
                g, b, hf = GUS[n]
                m = V[('m', sl_)][u]
                hh = g * 8 + hf * 4 + u
                if is0(i):
                    sx = s_scr[sl_, 0:(b + 1) * 128, u * 128:(u + 1) * 128]
                    tiles = range(b + 1)
                else:
                    sx = s_scr[sl_, :, u * 128:(u + 1) * 128]
                    for d in BITS:
                        sx = jnp.where(bitw[d], jnp.concatenate([sx[W - d * QS:], sx[:W - d * QS]], axis=0), sx)
                    tiles = [lin(i, NB, b - 2 + t) for t in range(3)]
                p = jnp.exp2(sx - m)
                lsum = None
                for c0 in range(0, p.shape[0], 128):
                    part = None
                    for j in range(c0 + 112, c0 - 1, -16):
                        part = p[j:j + 16] if part is None else part + p[j:j + 16]
                    lsum = part if lsum is None else lsum + part
                rl = pl.reciprocal(jnp.sum(lsum, axis=0, keepdims=True), approx=True)
                if not is0(i):
                    pm = p[0:128]
                    p = jnp.concatenate([jnp.where(tri128, 0.0, pm), p[128:256], jnp.where(tri128, pm, 0.0)], axis=0)
                vw = upk(jnp.concatenate([vT_scr[t, hh * 8:(hh + 1) * 8, :] for t in tiles], axis=1))
                oT_scr[hh * 16:(hh + 1) * 16, b * 128:(b + 1) * 128] = dot(vw, p.astype(bf16)) * rl
                if u == 3 and n % 4 == 3:
                    o_scr[par(i), :, g * 128:(g + 1) * 128] = pk(oT_scr[g * 128:(g + 1) * 128, :].T.astype(bf16))

            def ffn(i, r0=0, nr=TQ, T=None):
                T = {} if T is None else T

                def get_o():
                    if 'o' not in T:
                        T['o'] = Lhs(o_scr[par(i), r0 // 2:(r0 + nr) // 2, :])
                        T['x1'] = []
                    return T['o']

                def fin_wo(j, attn):
                    xp = x_v[lin(i, 1, 0), r0:r0 + nr, j * 128:(j + 1) * 128].astype(f32)
                    T['x1'].append(xp + mod(2, j * 128, (j + 1) * 128) * attn)
                    if j == 3 and kind != 'first':
                        get_h2()

                def get_h2():
                    if 'h2' not in T:
                        T['h2'] = Lhs(_ln(jnp.concatenate(T['x1'], axis=1)) * (1.0 + mod(4)) + mod(3))
                        T['a'] = []
                    return T['h2']

                def fin_w1(j, a):
                    T['a'].append(_silu(a))
                    if j % 4 == 3 or j == 13:
                        T[('ac', j // 4)] = Lhs(jnp.concatenate(T['a'][4 * (j // 4):j + 1], axis=1))

                def fin_w2r(pr, y):
                    T[('y', 2 * pr)] = y[:, 0:128]
                    T[('y', 2 * pr + 1)] = y[:, 128:256]

                def fin_w2(n, c, y):
                    T[('y', n)] = T[('y', n)] + y
                    if c == 2:
                        res = T['x1'][n] + mod(5, n * 128, (n + 1) * 128) * T[('y', n)]
                        if kind == 'last' and n == 3:
                            for a, b in ((0, 192), (192, 256)):
                                out_v[i, a:b, 384:512] = res[a:b].astype(bf16)
                                cp_out(i, 384, 128, a, b - a).start()
                            return
                        out_v[lin(i, 1, 0), r0:r0 + nr, n * 128:(n + 1) * 128] = res.astype(bf16)
                        if kind == 'last' and n == 2:
                            cp_out(i, 0, 384).start()
                        elif kind != 'last' and n == 3:
                            cp_out(lin(i, 1, 0)).start()

                items = [(get_o, P(slab, wo_ref, 0, D, j * 128, (j + 1) * 128), P(fin_wo, j)) for j in range(4)]
                items += [(get_h2, P(slab, w1_ref, 0, D, j * 128, (j + 1) * 128), P(fin_w1, j)) for j in range(14)]
                for pr in range(2):
                    items.append((P(T.get, ('ac', 3)), P(slab, w2_ref, 1536, F, pr * 256, (pr + 1) * 256),
                                  P(fin_w2r, pr)))
                    items += [(P(T.get, ('ac', c)), P(slab, w2_ref, c * 512, (c + 1) * 512, n * 128, (n + 1) * 128),
                               P(fin_w2, n, c)) for n in (2 * pr, 2 * pr + 1) for c in range(3)]
                return items

            def run(item):
                lhs, w, fin = item
                fin(dot(lhs().get(None), w()))

            def emit(order, blocks, streams, extra):
                stash = {}
                nq = npv = 0
                for ch in order:
                    if ch == 'Q':
                        a_qk(blocks[nq // NG], nq % NG, nq % NSLOT)
                        nq += 1
                    elif ch == '.':
                        q, u = divmod(npv, 4)
                        a_pv(blocks[q // NG], q % NG, q % NSLOT, u)
                        npv += 1
                    elif ch in streams:
                        run(streams[ch].pop(0))
                    elif ch.lower() in streams:
                        lhs, w, fin = streams[ch.lower()][0]
                        if ch not in stash:
                            stash[ch] = dot(lhs().get(0), w())
                        else:
                            streams[ch.lower()].pop(0)
                            fin(jnp.concatenate([stash.pop(ch), dot(lhs().get(1), w())], axis=0))
                    else:
                        extra[ch].pop(0)()

            if kind == 'first':
                groups = dma_groups()
                for grp in groups:
                    for c_ in grp:
                        c_.start()
                        pl.semaphore_signal(fence, 1)
                        pl.semaphore_wait(fence, 1)

                def wait(k):
                    for c_ in groups[k]:
                        c_.wait()

                def mod_a():
                    wait(1)
                    for j in range(8):
                        mod_chunk(j)

                wait(0)
                p_ln(0, mod_a)
                V[('h', 0)].get(None)
                wait(2)
                extra = {str(g): [P(p_skew, 0, g)] for g in range(4)}
                extra['w'] = [P(wait, k) for k in range(3, 7)]
                extra['m'] = [P(mod_chunk, j) for j in range(8, 24)]
                emit(order_first, (0, 1), dict(a=proj(0), b=proj(1), f=ffn(0)), extra)
                wait(7)
            elif kind == 'steady':
                bm1, b0, b1 = Blk(-1), Blk(0), Blk(1)
                p_ln(b0)
                emit(order_steady, (b0, b1), dict(a=proj(b0), b=proj(b1), f=ffn(bm1), g=ffn(b0)), {})
            else:
                Ta, Tb, T = {}, {}, {}
                a, b = ffn(NS - 1, 0, 128, Ta), ffn(NS - 1, 128, 128, Tb)
                for item in a[:4] + b[:4] + a[4:7] + b[4:7]:
                    run(item)
                T['h2'] = Lhs(jnp.concatenate([Ta['h2'].src, Tb['h2'].src], axis=0))
                for k in ('x1', 'a'):
                    T[k] = [jnp.concatenate(p, axis=0) for p in zip(Ta[k], Tb[k])]
                for item in ffn(NS - 1, T=T)[7:]:
                    run(item)
                cp(out_v, out_hbm, sem_o).wait()

        pl.when(step == 0)(lambda: region('first'))
        pl.when(jnp.logical_and(step > 0, step < 4))(lambda: region('steady'))
        pl.when(step == 4)(lambda: region('last'))

    def fn(A_x, A_wqkv, A_wo, B_x, B_w1, B_w2, c, w_mod):
        out = pl.pallas_call(
            kernel,
            grid=(5,),
            in_specs=[pl.BlockSpec(memory_space=pl.ANY)] * 7,
            out_specs=pl.BlockSpec(memory_space=pl.ANY),
            out_shape=jax.ShapeDtypeStruct((NS, TQ, D), bf16),
            scratch_shapes=[
                pltpu.VMEM((8, 6 * D), f32),
                pltpu.VMEM((4 * SL, S // 2, 128), u32),
                pltpu.VMEM((4, NH, 128), u32),
                pltpu.VMEM((4, HQ, 128), u32),
                pltpu.VMEM((S // 128, D // 2, 128), u32),
                pltpu.VMEM((2, D // 2, TQ), u32),
                pltpu.VMEM((D, TQ), f32),
                pltpu.VMEM((NSLOT, W, 512), f32),
                pltpu.VMEM((2, HQ, D), u32),
                pltpu.VMEM((NS, TQ, D), bf16),
                pltpu.VMEM((NS, TQ, D), bf16),
                pltpu.VMEM((D, 3 * D), bf16),
                pltpu.VMEM((D, D), bf16),
                pltpu.VMEM((D, F), bf16),
                pltpu.VMEM((F, D), bf16),
                pltpu.VMEM((1, D), bf16),
                pltpu.VMEM((D, 6 * D), bf16),
                pltpu.SemaphoreType.REGULAR,
                pltpu.SemaphoreType.DMA((8,)),
                pltpu.SemaphoreType.DMA,
            ],
            compiler_params=pltpu.CompilerParams(
                dimension_semantics=("arbitrary",),
                vmem_limit_bytes=100 * 2**20),
            name="fused",
            interpret=interpret,
        )(A_x.reshape(NS, TQ, D), A_wqkv, A_wo, B_w1, B_w2, c, w_mod)
        return out.reshape(1, S, D)
    return fn


_impl = make_kernel()


@jax.jit
def pallas_adaLN_cond__sliding_block__dense_activation_silu__prompt_kernel(
    A_x: jax.Array,
    A_wqkv: jax.Array,
    A_wo: jax.Array,
    B_x: jax.Array,
    B_w1: jax.Array,
    B_w2: jax.Array,
    c: jax.Array,
    w_mod: jax.Array,
):
    return _impl(A_x, A_wqkv, A_wo, B_x, B_w1, B_w2, c, w_mod)
```
